```python
import os as _os
_os.environ.setdefault("JAX_PLATFORMS", "cpu")
import jax
import jax.numpy as jnp

def _softmax(x, axis=-1):
    return jax.nn.softmax(x, axis=axis)
def _gelu(x):
    return jax.nn.gelu(x, approximate=True)
def _silu(x):
    return jax.nn.silu(x)
def _sigmoid(x):
    return jax.nn.sigmoid(x)
def _layernorm(x, axis=-1, eps=1e-5):
    m = jnp.mean(x, axis=axis, keepdims=True)
    v = jnp.var(x, axis=axis, keepdims=True)
    return (x - m) / jnp.sqrt(v + eps)
def _scatter_add(tgt, idx, src, axis=0):
    return tgt.at[idx].add(src)
def _segment_sum(src, seg, n):
    return jax.ops.segment_sum(src, seg, n)
class _Rng:
    def __init__(self, key):
        self._k = key
    def _next(self):
        self._k, sub = jax.random.split(self._k)
        return sub
    def normal(self, shape):
        return jax.random.normal(self._next(), shape, dtype=jnp.bfloat16)
    def randint(self, lo, hi, shape):
        return jax.random.randint(self._next(), shape, lo, hi, dtype=jnp.int32)
    def uniform(self, shape, lo=0.0, hi=1.0):
        return jax.random.uniform(self._next(), shape, jnp.bfloat16, lo, hi)
    def permutation(self, n):
        return jax.random.permutation(self._next(), n)


kernel_name = 'parallel_sum__ssm_conv_s4__mixer_channel_mlp__prompt'

def setup_inputs():
    _rng = _Rng(jax.random.key(int.from_bytes(__import__("os").urandom(4), "little")))
    _w = (lambda a: (lambda t: t.astype(jnp.bfloat16) if jnp.issubdtype(t.dtype, jnp.floating) else t)(jnp.asarray(a)))
    def _A_setup():
        B, L, D, N = 1, 2048, 512, 128
        A_re = -jnp.exp((lambda *s: _rng.normal(s) * 0.1)(D, N))
        A_im = jnp.pi * (lambda *s: _rng.normal(s) * 0.1)(D, N)
        B_re = (lambda *s: _rng.normal(s) * 0.1)(D, N)
        B_im = (lambda *s: _rng.normal(s) * 0.1)(D, N)
        C_re = (lambda *s: _rng.normal(s) * 0.1)(D, N)
        C_im = (lambda *s: _rng.normal(s) * 0.1)(D, N)
        log_dt = (lambda *s: _rng.normal(s) * 0.1)(D) * 0.5 - 4.0
        Dskip = (lambda *s: _rng.normal(s) * 0.05)(D)
        return {
            "u": _w((lambda *s: _rng.normal(s) * 0.05)(B, L, D)),
            "A_re": _w(A_re),
            "A_im": _w(A_im),
            "B_re": _w(B_re),
            "B_im": _w(B_im),
            "C_re": _w(C_re),
            "C_im": _w(C_im),
            "log_dt": _w(log_dt),
            "Dskip": _w(Dskip),
        }
    _A_in = _A_setup()

    def _B_setup():
        B, S, D, F = 1, 2048, 512, 1792
        return {
            "x": _w((lambda *s: _rng.normal(s) * 0.05)(B, S, D)),
            "w1": _w((lambda *s: _rng.normal(s) * 0.2)(D, F) * (D ** -0.5)),
            "b1": _w((lambda *s: _rng.normal(s) * 0.2)(F)),
            "w2": _w((lambda *s: _rng.normal(s) * 0.2)(F, D) * (F ** -0.5)),
            "b2": _w((lambda *s: _rng.normal(s) * 0.05)(D)),
        }
    _B_in = _B_setup()

    return {
        "A_u": _A_in["u"],
        "A_A_re": _A_in["A_re"],
        "A_A_im": _A_in["A_im"],
        "A_B_re": _A_in["B_re"],
        "A_B_im": _A_in["B_im"],
        "A_C_re": _A_in["C_re"],
        "A_C_im": _A_in["C_im"],
        "A_log_dt": _A_in["log_dt"],
        "A_Dskip": _A_in["Dskip"],
        "B_x": _B_in["x"],
        "B_w1": _B_in["w1"],
        "B_b1": _B_in["b1"],
        "B_w2": _B_in["w2"],
        "B_b2": _B_in["b2"],
    }

def reference(A_u, A_A_re, A_A_im, A_B_re, A_B_im, A_C_re, A_C_im, A_log_dt, A_Dskip, B_x, B_w1, B_b1, B_w2, B_b2):
    def _A_ref(u, A_re, A_im, B_re, B_im, C_re, C_im, log_dt, Dskip):
        Bsz, L, D = u.shape
        dt = jnp.exp(log_dt)[:, None]
        A = A_re + 1j * A_im
        Bc = B_re + 1j * B_im
        Cc = C_re + 1j * C_im
        logdA = dt * A
        dB = dt * Bc
        l = (lambda x, dt: x.astype(dt))(jnp.arange(L), A_re.dtype)
        P = jnp.exp(logdA[:, :, None] * l[None, None, :])
        K = jnp.einsum("dn,dnl,dn->dl", Cc, P, dB).real
        L2 = 2 * L
        Kp = jnp.pad(K, ((0, 0), (0, L)))
        up = (lambda x, *d: x.transpose(*d))(u, 0, 2, 1)
        up = jnp.pad(up, ((0, 0), (0, 0), (0, L)))
        Kf = (lambda x, axes=(-2,-1): jnp.fft.rfft2(x.astype(jnp.float32), axes=axes))(Kp[:, None, :], axes=(-2, -1))
        Uf = (lambda x, axes=(-2,-1): jnp.fft.rfft2(x.astype(jnp.float32), axes=axes))(up[:, :, None, :], axes=(-2, -1))
        Yf = Uf * Kf[None, :, :, :]
        y = (lambda x, s, axes=(-2,-1): jnp.fft.irfft2(x, s=s, axes=axes).astype(jnp.bfloat16))(Yf, (1, L2), axes=(-2, -1))[:, :, 0, :L]
        y = (lambda x, *d: x.transpose(*d))(y, 0, 2, 1) + u * Dskip[None, None, :]
        return y

    def _B_ref(x, w1, b1, w2, b2):
        y = _layernorm(x, axis=-1)
        h = _gelu(jnp.einsum("bsd,df->bsf", y, w1) + b1)
        return jnp.einsum("bsf,fd->bsd", h, w2) + b2

    x = A_u
    xn = _layernorm(x, axis=-1)
    return x + _A_ref(xn, A_A_re, A_A_im, A_B_re, A_B_im, A_C_re, A_C_im, A_log_dt, A_Dskip) + _B_ref(xn, B_w1, B_b1, B_w2, B_b2)
```

```python
import jax
import jax.numpy as jnp
import jax.experimental.pallas as pl
import jax.experimental.pallas.tpu as pltpu

F32 = jnp.float32
BF16 = jnp.bfloat16

L, D, NS, FF = 2048, 512, 128, 1792
BLK = 128
NB = L // BLK
TM = 256
SPB = TM // BLK
CH = 128
NG = CH // 8

ALPH = [[16 * m for m in range(16)],
        [32 * m for m in range(8, 16)],
        [64 * m for m in range(8, 16)],
        [128 * m for m in range(8, 16)] + [2048]]
ROW0 = [0, 16, 24, 32]
NROWP = 48


def _tile_of(e, m):
    if e == 0:
        return m // 8, m % 8
    if m < 8:
        return e + 1, m
    return 5, 0


def _blocks_tiles():
    import numpy as np
    lam = np.arange(L, dtype=np.float32)
    u = lam.view(np.uint32)
    lam = ((u + 0x7FFF + ((u >> 16) & 1)) & 0xFFFF0000).astype(np.uint32).view(np.float32)
    out = []
    for i in range(NB):
        tiles = set()
        for v in lam[i * BLK:(i + 1) * BLK]:
            v = int(v)
            if v < 128:
                tiles.add(0)
            elif v >= 2048:
                tiles.add(5)
            else:
                t = 1
                while v >= 128 * 2 ** t:
                    t += 1
                tiles.add(t)
        out.append(sorted(tiles))
    return out


BLOCK_TILES = _blocks_tiles()


def _cmul(ar, ai, br, bi):
    return ar * br - ai * bi, ar * bi + ai * br


def _csq(ar, ai):
    return ar * ar - ai * ai, 2.0 * ar * ai


def _cexp(xr, xi):
    m = jnp.exp(xr)
    return m * jnp.cos(xi), m * jnp.sin(xi)


def _layernorm_bf16(x):
    xf = x.astype(F32)
    mu = jnp.mean(xf, axis=-1, keepdims=True)
    var = jnp.mean(jnp.square(xf - mu), axis=-1, keepdims=True)
    m = mu.astype(BF16).astype(F32)
    v = var.astype(BF16).astype(F32)
    den = jnp.sqrt((v + 1e-5).astype(BF16).astype(F32)).astype(BF16).astype(F32)
    num = (xf - m).astype(BF16).astype(F32)
    return (num / den).astype(BF16)


def _kernel(x_ref, are_ref, aim_ref, bre_ref, bim_ref, cre_ref, cim_ref, ldt_ref,
            dsk_ref, w1_ref, b1_ref, w2_ref, b2_ref, o_ref,
            ffwd_ref, finv_ref, kf_ref, wf_ref, uprev_ref,
            ktab_ref, lhs_ref, rhs_ref, rev_ref, xn_ref, snap_ref, yf_ref):
    step = pl.program_id(0)

    @pl.when(step == 0)
    def _setup():
        row = jax.lax.broadcasted_iota(jnp.int32, (2 * BLK, BLK), 0)
        col = jax.lax.broadcasted_iota(jnp.int32, (2 * BLK, BLK), 1)
        fr = row % BLK
        ph = (((2 * fr + 1) * col) % (4 * BLK)).astype(F32) * (jnp.pi / (2 * BLK))
        ffwd = jnp.where(row < BLK, jnp.cos(ph), -jnp.sin(ph))
        ffwd_ref[...] = ffwd.astype(BF16)
        row2 = jax.lax.broadcasted_iota(jnp.int32, (BLK, 2 * BLK), 0)
        col2 = jax.lax.broadcasted_iota(jnp.int32, (BLK, 2 * BLK), 1)
        fc = col2 % BLK
        ph2 = (((2 * fc + 1) * (row2 + BLK)) % (4 * BLK)).astype(F32) * (jnp.pi / (2 * BLK))
        finv = jnp.where(col2 < BLK, jnp.cos(ph2), -jnp.sin(ph2)) * (1.0 / BLK)
        finv_ref[...] = finv.astype(BF16)
        uprev_ref[...] = jnp.zeros(uprev_ref.shape, F32)

        lane8 = jax.lax.broadcasted_iota(jnp.int32, (8, 128), 1) % 8

        def chunk(cidx, carry):
            r0 = pl.multiple_of(cidx * CH, CH)
            rows = pl.ds(r0, CH)
            ld = lambda ref: ref[rows, :].astype(F32)
            dt = jnp.exp(ldt_ref[rows, :].astype(F32)).astype(BF16).astype(F32)
            zr = dt * ld(are_ref)
            zi = dt * ld(aim_ref)
            dbr = dt * ld(bre_ref)
            dbi = dt * ld(bim_ref)
            cr, ci = _cmul(ld(cre_ref), ld(cim_ref), dbr, dbi)
            w1r, w1i = _cexp(zr, zi)
            for s in range(8):
                rev_ref[0, pl.ds(7 - s, NG, stride=8), :] = w1r.reshape(NG, 8, 128)[:, s, :]
                rev_ref[1, pl.ds(7 - s, NG, stride=8), :] = w1i.reshape(NG, 8, 128)[:, s, :]
            pw = {1: (rev_ref[0], rev_ref[1])}
            need = sorted(set((2 ** e) * b for e in range(4) for b in range(16)) - {0, 1})
            for k in need:
                if k % 2 == 0 and k // 2 in pw:
                    pw[k] = _csq(*pw[k // 2])
                else:
                    pw[k] = _cmul(*pw[k - 1], *pw[1])
            ones = jnp.ones((CH, 128), F32)
            zeros = jnp.zeros((CH, 128), F32)
            for e in range(4):
                for b2 in range(8):
                    parts_r, parts_i = [], []
                    for b in (2 * b2, 2 * b2 + 1):
                        k = (2 ** e) * b
                        pr, pi_ = (ones, zeros) if k == 0 else pw[k]
                        parts_r.append(pr.reshape(NG, 8, 128))
                        parts_i.append(pi_.reshape(NG, 8, 128))
                    rhs_ref[e, :, 16 * b2:16 * b2 + 16, 0:128] = jnp.concatenate(parts_r, axis=1).astype(BF16)
                    rhs_ref[e, :, 16 * b2:16 * b2 + 16, 128:256] = jnp.concatenate(parts_i, axis=1).astype(BF16)
            w16 = _cexp(zr * 16.0, zi * 16.0)
            w256 = _cexp(zr * 256.0, zi * 256.0)
            w32 = _csq(*w16)
            w64 = _csq(*w32)
            w128 = _csq(*w64)
            w512 = _csq(*w256)
            w1024 = _csq(*w512)
            w2048 = _csq(*w1024)
            starts = [(cr, ci), _cmul(cr, ci, *w256), _cmul(cr, ci, *w512), _cmul(cr, ci, *w1024)]
            steps = [w16, w32, w64, w128]
            e1 = []
            for e in range(4):
                cur = starts[e]
                for m in range(8 if e else 16):
                    if m:
                        cur = _cmul(*cur, *steps[e])
                    e1.append(cur)
            e1.append(_cmul(cr, ci, *w2048))
            e1.append((zeros, zeros))
            for r2 in range(len(e1) // 2):
                pa, pb = e1[2 * r2], e1[2 * r2 + 1]
                lhs_ref[:, 16 * r2:16 * r2 + 16, 0:128] = jnp.concatenate(
                    [pa[0].reshape(NG, 8, 128), pb[0].reshape(NG, 8, 128)], axis=1).astype(BF16)
                lhs_ref[:, 16 * r2:16 * r2 + 16, 128:256] = jnp.concatenate(
                    [(-pa[1]).reshape(NG, 8, 128), (-pb[1]).reshape(NG, 8, 128)], axis=1).astype(BF16)

            def group(g, c2):
                tiles = [jnp.zeros((8, 128), F32) for _ in range(6)]
                for e in range(4):
                    nrow = len(ALPH[e])
                    mpad = 8 * nrow if nrow % 2 == 0 else 8 * (nrow + 1)
                    lhs = lhs_ref[g, 8 * ROW0[e]:8 * ROW0[e] + mpad, :]
                    raw = jax.lax.dot_general(lhs, rhs_ref[e, g], (((1,), (1,)), ((), ())),
                                              preferred_element_type=F32)
                    for m in range(nrow):
                        t, al = _tile_of(e, m)
                        rolled = pltpu.roll(raw[8 * m:8 * m + 8, :], al + 1, 1, stride=1, stride_axis=0)
                        tiles[t] = jnp.where(lane8 == al, rolled, tiles[t])
                rr = pl.multiple_of(r0 + g * 8, 8)
                for t in range(6):
                    ktab_ref[pl.ds(rr, 8), 128 * t:128 * (t + 1)] = tiles[t]
                return c2

            jax.lax.fori_loop(0, NG, group, 0, unroll=NG)
            return carry

        jax.lax.fori_loop(0, D // CH, chunk, 0)

        tau = jax.lax.broadcasted_iota(jnp.int32, (BLK, BLK), 0)
        jj = jax.lax.broadcasted_iota(jnp.int32, (BLK, BLK), 1)
        slot_al = jj % 8
        slot_b = (jj // 8 + 15) % 16
        slot_m = 16 * slot_al + slot_b
        ffwd_b = ffwd_ref[...]
        for i in range(NB):
            lam = (tau + i * BLK).astype(F32).astype(BF16).astype(F32)
            acc = None
            for t in BLOCK_TILES[i]:
                if t == 0:
                    tl = slot_m
                elif t < 5:
                    tl = (2 ** (t - 1)) * (128 + slot_m)
                else:
                    tl = jnp.where(slot_al == 0, 2048 + 8 * slot_b, -1)
                sel = (lam == tl.astype(F32)).astype(BF16)
                phi = jnp.dot(ffwd_b, sel, preferred_element_type=F32).astype(BF16)
                kt = ktab_ref[:, 128 * t:128 * (t + 1)].astype(BF16)
                part = jax.lax.dot_general(phi, kt, (((1,), (1,)), ((), ())), preferred_element_type=F32)
                acc = part if acc is None else acc + part
            kf_ref[i] = acc

        sgn = 1.0 - 2.0 * (jax.lax.broadcasted_iota(jnp.int32, (BLK, 1), 0) % 2).astype(F32)
        snap_ref[...] = jnp.zeros(snap_ref.shape, F32)

        def fwd(j, carry):
            rj = pl.multiple_of(j * BLK, BLK)
            xn_j = _layernorm_bf16(x_ref[pl.ds(rj, BLK), :])
            xn_ref[pl.ds(rj, BLK), :] = xn_j
            uf = jnp.dot(ffwd_b, xn_j, preferred_element_type=F32)
            up = uprev_ref[...]
            wf_ref[j, 0:BLK, :] = up[0:BLK] + sgn * uf[BLK:2 * BLK]
            wf_ref[j, BLK:2 * BLK, :] = up[BLK:2 * BLK] - sgn * uf[0:BLK]
            uprev_ref[...] = uf
            return carry

        jax.lax.fori_loop(0, NB, fwd, 0)

    pb = NB - 1 - step
    RC = 16
    for r0 in range(0, BLK, RC):
        ar = jnp.zeros((RC, D), F32)
        ai = jnp.zeros((RC, D), F32)
        for t in range(NB + 1):
            first = t <= step
            ik = jnp.where(first, t, t - step - 1)
            iw = jnp.where(first, step - t, NB - t)
            kr = kf_ref[ik, r0:r0 + RC, :]
            ki = kf_ref[ik, BLK + r0:BLK + r0 + RC, :]
            wr = wf_ref[iw, r0:r0 + RC, :]
            wi = wf_ref[iw, BLK + r0:BLK + r0 + RC, :]
            ar = ar + (kr * wr - ki * wi)
            ai = ai + (kr * wi + ki * wr)
            if t < NB:
                slot = jnp.where(t == step, 1, 0)
                snap_ref[slot, r0:r0 + RC, :] = ar
                snap_ref[slot, BLK + r0:BLK + r0 + RC, :] = ai
        yf_ref[1, r0:r0 + RC, :] = ar - snap_ref[1, r0:r0 + RC, :]
        yf_ref[1, BLK + r0:BLK + r0 + RC, :] = ai - snap_ref[1, BLK + r0:BLK + r0 + RC, :]
    finv = finv_ref[...]
    ya_f = jnp.dot(finv, snap_ref[1].astype(BF16), preferred_element_type=F32)
    yb_f = jnp.dot(finv, yf_ref[1].astype(BF16), preferred_element_type=F32)
    yconv = jnp.concatenate([ya_f, yb_f], axis=0).astype(BF16)

    ra = pl.multiple_of(step * BLK, BLK)
    rb = pl.multiple_of(pb * BLK, BLK)
    x = jnp.concatenate([x_ref[pl.ds(ra, BLK), :], x_ref[pl.ds(rb, BLK), :]], axis=0)
    xn = jnp.concatenate([xn_ref[pl.ds(ra, BLK), :], xn_ref[pl.ds(rb, BLK), :]], axis=0)
    ya = (yconv.astype(F32) + (xn.astype(F32) * dsk_ref[...].astype(F32)).astype(BF16).astype(F32)).astype(BF16)

    y2 = _layernorm_bf16(xn)
    h = jnp.dot(y2, w1_ref[...], preferred_element_type=F32).astype(BF16)
    h = (h.astype(F32) + b1_ref[...].astype(F32)).astype(BF16).astype(F32)
    h = jax.nn.gelu(h, approximate=True).astype(BF16)
    yb = jnp.dot(h, w2_ref[...], preferred_element_type=F32).astype(BF16)
    yb = (yb.astype(F32) + b2_ref[...].astype(F32)).astype(BF16)

    out = (x.astype(F32) + ya.astype(F32)).astype(BF16)
    out = (out.astype(F32) + yb.astype(F32)).astype(BF16)
    o_ref[pl.ds(ra, BLK), :] = out[0:BLK]
    o_ref[pl.ds(rb, BLK), :] = out[BLK:2 * BLK]


@jax.jit
def pallas_parallel_sum__ssm_conv_s4__mixer_channel_mlp__prompt_kernel(
    A_u: jax.Array,
    A_A_re: jax.Array,
    A_A_im: jax.Array,
    A_B_re: jax.Array,
    A_B_im: jax.Array,
    A_C_re: jax.Array,
    A_C_im: jax.Array,
    A_log_dt: jax.Array,
    A_Dskip: jax.Array,
    B_x: jax.Array,
    B_w1: jax.Array,
    B_b1: jax.Array,
    B_w2: jax.Array,
    B_b2: jax.Array,
):
    x = A_u.reshape(L, D)
    full = lambda shape: pl.BlockSpec(shape, lambda i: (0,) * len(shape))
    out = pl.pallas_call(
        _kernel,
        grid=(NB // 2,),
        in_specs=[full((L, D))]
        + [full((D, NS))] * 6
        + [full((D, 1)), full((1, D)), full((D, FF)), full((1, FF)), full((FF, D)), full((1, D))],
        out_specs=full((L, D)),
        out_shape=jax.ShapeDtypeStruct((L, D), BF16),
        scratch_shapes=[
            pltpu.VMEM((2 * BLK, BLK), BF16),
            pltpu.VMEM((BLK, 2 * BLK), BF16),
            pltpu.VMEM((NB, 2 * BLK, D), F32),
            pltpu.VMEM((NB, 2 * BLK, D), F32),
            pltpu.VMEM((2 * BLK, D), F32),
            pltpu.VMEM((D, 6 * 128), F32),
            pltpu.VMEM((NG, 8 * NROWP, 256), BF16),
            pltpu.VMEM((4, NG, 128, 256), BF16),
            pltpu.VMEM((2, CH, 128), F32),
            pltpu.VMEM((L, D), BF16),
            pltpu.VMEM((2, 2 * BLK, D), F32),
            pltpu.VMEM((2, 2 * BLK, D), F32),
        ],
        compiler_params=pltpu.CompilerParams(
            dimension_semantics=("arbitrary",),
            vmem_limit_bytes=100 * 2 ** 20),
    )(x, A_A_re, A_A_im, A_B_re, A_B_im, A_C_re, A_C_im,
      A_log_dt.reshape(D, 1), A_Dskip.reshape(1, D),
      B_w1, B_b1.reshape(1, FF), B_w2, B_b2.reshape(1, D))
    return out.reshape(1, L, D)
```
